```python
import jax
import jax.numpy as jnp

def _softmax(x, axis=-1):
    return jax.nn.softmax(x, axis=axis)
def _gelu(x):
    return jax.nn.gelu(x, approximate=True)
def _silu(x):
    return jax.nn.silu(x)
def _sigmoid(x):
    return jax.nn.sigmoid(x)
def _layernorm(x, axis=-1, eps=1e-5):
    m = jnp.mean(x, axis=axis, keepdims=True)
    v = jnp.var(x, axis=axis, keepdims=True)
    return (x - m) / jnp.sqrt(v + eps)
def _scatter_add(tgt, idx, src, axis=0):
    return tgt.at[idx].add(src)
def _segment_sum(src, seg, n):
    return jax.ops.segment_sum(src, seg, n)
class _Rng:
    def __init__(self, key):
        self._k = key
    def _next(self):
        self._k, sub = jax.random.split(self._k)
        return sub
    def normal(self, shape):
        return jax.random.normal(self._next(), shape, dtype=jnp.bfloat16)
    def randint(self, lo, hi, shape):
        return jax.random.randint(self._next(), shape, lo, hi, dtype=jnp.int32)
    def uniform(self, shape, lo=0.0, hi=1.0):
        return jax.random.uniform(self._next(), shape, jnp.bfloat16, lo, hi)
    def permutation(self, n):
        return jax.random.permutation(self._next(), n)


kernel_name = 'gated_mix__softmax_full_mha__glu_gated_bilinear__prompt'

def _fwd_setup_inputs():
    _rng = _Rng(jax.random.key(int.from_bytes(__import__("os").urandom(4), "little")))
    _w = (lambda a: (lambda t: t.astype(jnp.bfloat16) if jnp.issubdtype(t.dtype, jnp.floating) else t)(jnp.asarray(a)))
    def _A_setup():
        B, S, D = 1, 2048, 1024
        return {
            "x": _w((lambda *s: _rng.normal(s) * 0.05)(B, S, D)),
            "wqkv": _w((lambda *s: _rng.normal(s) * 0.05)(D, 3 * D)),
            "wo": _w((lambda *s: _rng.normal(s) * 0.05)(D, D)),
        }
    _A_in = _A_setup()

    def _B_setup():
        B, S, D, F = 1, 2048, 1024, 3584
        return {
            "x": _w((lambda *s: _rng.normal(s) * 0.05)(B, S, D)),
            "w_gate": _w((lambda *s: _rng.normal(s) * 0.05)(D, F) * (D ** -0.5)),
            "w_up": _w((lambda *s: _rng.normal(s) * 0.05)(D, F) * (D ** -0.5)),
            "w_down": _w((lambda *s: _rng.normal(s) * 0.05)(F, D) * (F ** -0.5)),
        }
    _B_in = _B_setup()

    return {
        "A_x": _A_in["x"],
        "A_wqkv": _A_in["wqkv"],
        "A_wo": _A_in["wo"],
        "B_x": _B_in["x"],
        "B_w_gate": _B_in["w_gate"],
        "B_w_up": _B_in["w_up"],
        "B_w_down": _B_in["w_down"],
        "gate_w": _w((lambda *s: _rng.normal(s) * 0.05)(1024)),
    }

def _fwd_reference(A_x, A_wqkv, A_wo, B_x, B_w_gate, B_w_up, B_w_down, gate_w):
    def _A_ref(x, wqkv, wo):
        B, S, D = x.shape
        H = 32; Dh = D // H
        qkv = (lambda x, *d: x.transpose(*d))((x @ wqkv).reshape(B, S, 3, H, Dh), 2, 0, 3, 1, 4)
        q, k, v = qkv[0], qkv[1], qkv[2]
        scale = Dh ** -0.5
        scores = jnp.einsum("bhqd,bhkd->bhqk", q, k) * scale
        p = _softmax(scores, axis=-1)
        o = jnp.einsum("bhqk,bhkd->bhqd", p, v)
        return (lambda x, *d: x.transpose(*d))(o, 0, 2, 1, 3).reshape(B, S, D) @ wo

    def _B_ref(x, w_gate, w_up, w_down):
        g = jnp.einsum("bsd,df->bsf", x, w_gate)
        u = jnp.einsum("bsd,df->bsf", x, w_up)
        h = g * u
        return jnp.einsum("bsf,fd->bsd", h, w_down)

    x = A_x
    g = _sigmoid((x * gate_w).sum(-1, keepdims=True))
    a = _A_ref(x, A_wqkv, A_wo)
    b = _B_ref(x, B_w_gate, B_w_up, B_w_down)
    return g * a + (1 - g) * b


def setup_inputs():
    _inp = _fwd_setup_inputs()
    _gk = jax.random.fold_in(jax.random.key(int.from_bytes(__import__("os").urandom(4), "little")), 2**31 - 1)
    _shapes = [[1, 2048, 1024]]
    _dtypes = ['bfloat16']
    _gks = jax.random.split(_gk, len(_shapes))
    _gs = [jax.random.normal(k, s, dtype=jnp.dtype(d)) * 0.05 for k, s, d in zip(_gks, _shapes, _dtypes)]
    _inp["grad_out"] = _gs[0]
    return _inp

def reference(A_x, A_wqkv, A_wo, B_w_gate, B_w_up, B_w_down, gate_w, B_x, grad_out):
    _const = dict(B_x=B_x)
    def _f(*_d):
        return _fwd_reference(**{'A_x': _d[0], 'A_wqkv': _d[1], 'A_wo': _d[2], 'B_w_gate': _d[3], 'B_w_up': _d[4], 'B_w_down': _d[5], 'gate_w': _d[6], **_const})
    _out, _vjp = jax.vjp(_f, A_x, A_wqkv, A_wo, B_w_gate, B_w_up, B_w_down, gate_w)
    _grads = _vjp(grad_out)
    _out0 = jnp.asarray(_out)
    return (_out0, *[jnp.asarray(_g) for _g in _grads])
```

```python
import math

import jax
import jax.numpy as jnp
import jax.experimental.pallas as pl
import jax.experimental.pallas.tpu as pltpu

S, D, F, H, DH = 2048, 1024, 3584, 32, 32
R = 512
NR = S // R
FC = 512
NF = F // FC
WS = 16
R4 = 512
NR4 = S // R4
TQ = R
CK = 128
NC = S // CK
CPB = R // CK
SCALE = DH ** -0.5
LOG2E = math.log2(math.e)
LN2 = math.log(2.0)
BF16, F32 = jnp.bfloat16, jnp.float32

_NN = (((1,), (0,)), ((), ()))
_NT = (((1,), (1,)), ((), ()))
_TN = (((0,), (0,)), ((), ()))
_TT = (((0,), (1,)), ((), ()))


def _dot(a, b, dn):
    return jax.lax.dot_general(a, b, dn, preferred_element_type=F32)


def _blocks(z):
    m, n = z.shape
    return z[:m // 2, :n // 2], z[:m // 2, n // 2:], z[m // 2:, :n // 2], z[m // 2:, n // 2:]


def _full(c11, c12, c21, c22):
    return jnp.concatenate([jnp.concatenate([c11, c12], axis=1),
                            jnp.concatenate([c21, c22], axis=1)], axis=0)


def _nset(z):
    a, b, c, d = _blocks(z)
    return [(a + d).astype(BF16), (c + d).astype(BF16), (a + b).astype(BF16),
            (c - a).astype(BF16), (b - d).astype(BF16)]


def _tset(z):
    a, b, c, d = _blocks(z)
    return [(a + d).astype(BF16), (b + d).astype(BF16), (a + c).astype(BF16),
            (b - a).astype(BF16), (c - d).astype(BF16)]


def _lhs7(z11, z22, s):
    return [s[0], s[1], z11, z22, s[2], s[3], s[4]]


def _rhs7(z11, z22, s):
    return [s[0], z11, s[4], s[3], z22, s[2], s[1]]


def _rhs7_t(z11, z22, t):
    return [t[0], z11, t[4], t[3], z22, t[2], t[1]]


class _Strassen:
    ORDER = (1, 4, 2, 3, 0, 5, 6)

    def __init__(self, lhs, rhs, dn, swap=False):
        self.lhs, self.rhs, self.dn, self.swap = lhs, rhs, dn, swap
        self.m = [None] * 7
        self.done = 0

    def prod(self, n=7):
        for i in self.ORDER[self.done:self.done + n]:
            self.m[i] = (_dot(self.rhs[i], self.lhs[i], self.dn) if self.swap
                         else _dot(self.lhs[i], self.rhs[i], self.dn))
        self.done = min(7, self.done + n)
        return self

    def blocks(self):
        self.prod()
        m1, m2, m3, m4, m5, m6, m7 = self.m
        if self.swap:
            return m1 + m4 - m5 + m7, m2 + m4, m3 + m5, m1 - m2 + m3 + m6
        return m1 + m4 - m5 + m7, m3 + m5, m2 + m4, m1 - m2 + m3 + m6


def _strassen(lhs, rhs, dn, swap=False):
    return _Strassen(lhs, rhs, dn, swap).blocks()


class _NoScope:
    def __enter__(self):
        return self

    def __exit__(self, *exc):
        return False


def _scope(name):
    del name
    return _NoScope()


def _loop(name, n, body, init=0):
    with _scope(name):
        return jax.lax.fori_loop(0, n, body, init)


def _rows(r, n=R):
    return pl.ds(pl.multiple_of(r * n, n), n)


def _kernel(x_hbm, wqkv_hbm, wo_hbm, wg_hbm, wu_hbm, wd_hbm, gw_ref, dout_hbm,
            out_hbm, dx_hbm, dwqkv_hbm, dwo_hbm, dwg_hbm, dwu_hbm, dwd_hbm, dgw_ref,
            x_v, dout_v, wqkv_v, wo_v, wqs_v, wos_v, g_v, grow_v, ot_v, dqkvt_v, sem_in):
    def x_cp(r):
        return pltpu.make_async_copy(x_hbm.at[_rows(r)], x_v.at[_rows(r)], sem_in.at[r])

    def dout_cp(r):
        return pltpu.make_async_copy(dout_hbm.at[_rows(r)], dout_v.at[_rows(r)], sem_in.at[NR + r])

    wqkv_cp = pltpu.make_async_copy(wqkv_hbm, wqkv_v, sem_in.at[2 * NR])
    wo_cp = pltpu.make_async_copy(wo_hbm, wo_v, sem_in.at[2 * NR + 1])

    wo_cp.start()
    dout_cp(0).start()

    gw = gw_ref[0:1, :]

    def attn_scope(qt, kt, vt, dot_, kg, vg, s_scr, p_scr, m_scr, dl_scr, dob_scr):
        def clear_body(r, carry):
            dqkvt_v[r, D:3 * D, :] = jnp.zeros((2 * D, R), F32)
            return carry

        _loop("Clear", NR, clear_body)
        def wsum_loop(name, src, dst):
            def body(t, carry):
                top = pl.ds(pl.multiple_of(t * WS, WS), WS)
                bot = pl.ds(pl.multiple_of(D // 2 + t * WS, WS), WS)
                z = jnp.concatenate([src[top, :], src[bot, :]], axis=0).astype(F32)
                for i, v in enumerate(_nset(z)):
                    dst[i, top, :] = v
                return carry

            _loop(name, D // 2 // WS, body)

        with _scope("W0"):
            wo_cp.wait()
        for r in range(1, NR):
            dout_cp(r).start()
        wqkv_cp.start()
        for r in range(NR):
            x_cp(r).start()
        wsum_loop("Wsum0", wo_v, wos_v)
        gw8 = gw_ref[...].astype(BF16)

        def p1a_body(r, carry):
            dout_cp(r).wait()
            hd, hr = D // 2, R // 2
            dr = dout_v[_rows(r), :]
            dot_[r] = _full(*_strassen(
                _lhs7(wo_v[:hd, :hd], wo_v[hd:, hd:], [wos_v[i] for i in range(5)]),
                _rhs7_t(dr[:hr, :hd], dr[hr:, hd:], _tset(dr.astype(F32))), _NT)).astype(BF16)
            return carry

        _loop("P1a", NR, p1a_body)
        with _scope("W2"):
            for r in range(NR):
                x_cp(r).wait()
            wqkv_cp.wait()

        wsum_loop("Wsum1", wqkv_v, wqs_v)

        def p1b_body(r, carry):
            rows = _rows(r)
            xr = x_v[rows, :]
            hd, hr, hq = D // 2, R // 2, 3 * D // 2
            st = _Strassen(_lhs7(xr[:hr, :hd], xr[hr:, hd:], _nset(xr.astype(F32))),
                           _rhs7(wqkv_v[:hd, :hq], wqkv_v[hd:, hq:], [wqs_v[i] for i in range(5)]), _NN)
            st.prod(3)
            grow_v[r, 0:1, :] = jax.nn.sigmoid(_dot(gw8, xr, _NT)[0:1, :])
            qkv = _full(*st.blocks())
            q = (qkv[:, :D] * (SCALE * LOG2E)).astype(BF16)
            k = qkv[:, D:2 * D].astype(BF16)
            v = qkv[:, 2 * D:].astype(BF16)
            qt[r] = q.T
            kt[r] = k.T
            vt[r] = v.T
            for g in range(8):
                kg[g, rows, :] = k[:, g * 128:(g + 1) * 128]
                vg[g, rows, :] = v[:, g * 128:(g + 1) * 128]
            gate = jax.nn.sigmoid(jnp.sum(xr.astype(F32) * gw, axis=-1, keepdims=True))
            g_v[rows, :] = jnp.broadcast_to(gate, (R, 128))
            return carry

        _loop("P1b", NR, p1b_body)

        rowgrp = jax.lax.broadcasted_iota(jnp.int32, (128, TQ), 0) // 32

        def tidx(r0, c):
            return (c // CPB, pl.ds(r0, 32), slice((c % CPB) * CK, (c % CPB + 1) * CK))

        class StageA:
            def __init__(self, h, qb):
                self.g = h >> 2
                qg = qt[qb, pl.ds(pl.multiple_of(self.g * 128, 128), 128), :]
                self.wq = jnp.where(rowgrp == (h & 3), qg, jnp.zeros_like(qg))
                self.m = None

            def chunk(self, c):
                s = _dot(kg[self.g, c * CK:(c + 1) * CK, :], self.wq, _NN)
                s_scr[c * CK:(c + 1) * CK, :] = s
                mc = jnp.max(s.reshape(CK // 8, 8, TQ), axis=0)
                self.m = mc if self.m is None else jnp.maximum(self.m, mc)

            def fin(self):
                m_scr[0:1, :] = jnp.max(self.m, axis=0, keepdims=True)

        class StageB:
            def __init__(self, h, qb):
                self.qb = qb
                self.r0 = pl.multiple_of(h * 32, 32)
                self.m = m_scr[0:1, :]
                self.l = None
                self.o = None
                self.pb = {}

            def exp(self, c):
                p = jnp.exp2(s_scr[c * CK:(c + 1) * CK, :] - self.m)
                lc = jnp.sum(p.reshape(CK // 8, 8, TQ), axis=0)
                self.l = lc if self.l is None else self.l + lc
                p_scr[c * CK:(c + 1) * CK, :] = p
                self.pb[c] = p.astype(BF16)

            def pv(self, c):
                oc = _dot(vt[tidx(self.r0, c)], self.pb.pop(c), _NN)
                self.o = oc if self.o is None else self.o + oc

            def fin(self):
                inv = 1.0 / jnp.sum(self.l, axis=0, keepdims=True)
                o = self.o * inv
                ot_v[self.qb, pl.ds(self.r0, 32), :] = o.astype(BF16)
                do = dot_[self.qb, pl.ds(self.r0, 32), :].astype(F32) * grow_v[self.qb, 0:1, :]
                dl_scr[0:1, :] = jnp.sum(do * o, axis=0, keepdims=True) * inv
                dob_scr[...] = (do * inv).astype(BF16)

        class StageC:
            def __init__(self, h, qb):
                self.g = h >> 2
                self.qb = qb
                self.r0 = pl.multiple_of(h * 32, 32)
                self.rk = pl.multiple_of(D + h * 32, 32)
                self.rv = pl.multiple_of(2 * D + h * 32, 32)
                self.dob = dob_scr[...]
                do4 = jnp.concatenate([self.dob] * 4, axis=0)
                self.wdo = jnp.where(rowgrp == (h & 3), do4, jnp.zeros_like(do4))
                self.delta = dl_scr[0:1, :]
                self.qh = qt[qb, pl.ds(self.r0, 32), :]
                self.dq = None
                self.dp, self.ds, self.pb = {}, {}, {}

            def dpm(self, c):
                self.dp[c] = _dot(vg[self.g, c * CK:(c + 1) * CK, :], self.wdo, _NN)

            def dsv(self, c):
                p = p_scr[c * CK:(c + 1) * CK, :]
                self.pb[c] = p.astype(BF16)
                self.ds[c] = (p * (self.dp.pop(c) - self.delta)).astype(BF16)

            def dvm(self, c):
                dqkvt_v[tidx(self.rv, c)] += _dot(self.dob, self.pb.pop(c), _NT)

            def dqm(self, c):
                dqc = _dot(kt[tidx(self.r0, c)], self.ds.pop(c), _NN)
                self.dq = dqc if self.dq is None else self.dq + dqc

            def dkm(self, c):
                dqkvt_v[tidx(self.rk, c)] += _dot(self.qh, self.ds[c], _NT)

            def fin(self):
                dqkvt_v[self.qb, pl.ds(self.r0, 32), :] = self.dq * SCALE

        n_items = H * NR
        a = StageA(0, 0)
        for c in range(NC):
            a.chunk(c)
        a.fin()
        b = StageB(0, 0)
        a = StageA(1 // NR, 1 % NR)
        for c in range(NC):
            b.exp(c)
            b.pv(c)
            a.chunk(c)
        b.fin()
        a.fin()

        def attn_body(i, carry):
            i1 = jnp.minimum(i + 1, n_items - 1)
            i2 = jnp.minimum(i + 2, n_items - 1)
            cc = StageC(i >> 2, i & 3)
            b = StageB(i1 >> 2, i1 & 3)
            a = StageA(i2 >> 2, i2 & 3)
            cc.dpm(0)
            cc.dsv(0)
            b.exp(0)
            for c in range(NC):
                a.chunk(c)
                cc.dvm(c)
                if c + 1 < NC:
                    cc.dpm(c + 1)
                cc.dkm(c)
                b.pv(c)
                cc.dqm(c)
                if c + 1 < NC:
                    cc.dsv(c + 1)
                    b.exp(c + 1)
            cc.fin()
            b.fin()
            a.fin()
            return carry

        _loop("P2", n_items, attn_body)

    pl.run_scoped(
        attn_scope,
        pltpu.VMEM((NR, D, R), BF16), pltpu.VMEM((NR, D, R), BF16), pltpu.VMEM((NR, D, R), BF16),
        pltpu.VMEM((NR, D, R), BF16),
        pltpu.VMEM((8, S, 128), BF16), pltpu.VMEM((8, S, 128), BF16),
        pltpu.VMEM((S, TQ), F32), pltpu.VMEM((S, TQ), F32),
        pltpu.VMEM((8, TQ), F32), pltpu.VMEM((8, TQ), F32), pltpu.VMEM((32, TQ), BF16),
    )

    def tail_scope(bacc, dxacc, wgus, wds, dwgu_acc, dwd_acc, stg_gu, stg_d,
                   stg_q, stg_o, stg_out, stg_dx, sem_w, sem_dw, sem_q, sem_fin):
        def fcols(c):
            return pl.ds(pl.multiple_of(c * FC, FC), FC)

        def w_cps(c, slot):
            return (pltpu.make_async_copy(wg_hbm.at[:, fcols(c)], wgus.at[slot, :, 0:FC], sem_w.at[slot, 0]),
                    pltpu.make_async_copy(wu_hbm.at[:, fcols(c)], wgus.at[slot, :, FC:2 * FC], sem_w.at[slot, 1]),
                    pltpu.make_async_copy(wd_hbm.at[fcols(c), :], wds.at[slot], sem_w.at[slot, 2]))

        def dw_cps(c, slot):
            return (pltpu.make_async_copy(stg_gu.at[slot, :, 0:FC], dwg_hbm.at[:, fcols(c)], sem_dw.at[slot, 0]),
                    pltpu.make_async_copy(stg_gu.at[slot, :, FC:2 * FC], dwu_hbm.at[:, fcols(c)], sem_dw.at[slot, 1]),
                    pltpu.make_async_copy(stg_d.at[slot], dwd_hbm.at[fcols(c), :], sem_dw.at[slot, 2]))

        for cp in w_cps(0, 0):
            cp.start()

        otg = jnp.concatenate([(ot_v[r].astype(F32) * grow_v[r, 0:1, :]).astype(BF16) for r in range(NR)], axis=1)
        stg_o[...] = _dot(otg, dout_v[...], _NN).astype(BF16)
        dwo_cp = pltpu.make_async_copy(stg_o, dwo_hbm, sem_q.at[2])
        dwo_cp.start()

        def q_cp(j, slot):
            return pltpu.make_async_copy(
                stg_q.at[slot], dwqkv_hbm.at[:, pl.ds(pl.multiple_of(j * R, R), R)], sem_q.at[slot])

        def p3_body(j, carry):
            slot = j % 2

            @pl.when(j >= 2)
            def _():
                q_cp(j - 2, slot).wait()

            rows = _rows(j)
            hd, hr, hs = D // 2, R // 2, S // 2
            dt = jnp.concatenate([dqkvt_v[r, rows, :] for r in range(NR)], axis=1)
            blk = _full(*_strassen(
                _lhs7(dt[:hr, :hs].astype(BF16), dt[hr:, hs:].astype(BF16), _nset(dt)),
                _rhs7(x_v[:hs, :hd], x_v[hs:, hd:], _nset(x_v[...].astype(F32))), _NN))
            blk = blk * jnp.where(j // 2 == 1, LN2, 1.0)
            stg_q[slot] = blk.astype(BF16).T
            q_cp(j, slot).start()
            return carry

        n_j = 3 * D // R
        _loop("P3", n_j, p3_body)

        def p4_body(it, carry):
            c = it // NR4
            r = it % NR4
            slot = c % 2

            @pl.when(r == 0)
            def _():
                for cp in w_cps(c, slot):
                    cp.wait()

                @pl.when(c + 1 < NF)
                def _():
                    for cp in w_cps(c + 1, 1 - slot):
                        cp.start()

                @pl.when(c >= 2)
                def _():
                    for cp in dw_cps(c - 2, slot):
                        cp.wait()

            hd, hf, hr = D // 2, FC // 2, R4 // 2
            rows = _rows(r, R4)
            top = pl.ds(pl.multiple_of(r * R4, R4), hr)
            bot = pl.ds(pl.multiple_of(r * R4 + hr, hr), hr)
            w, wd = wgus.at[slot], wds.at[slot]

            wd11, wd22 = wd[:hf, :hd], wd[hf:, hd:]
            wds_ = _nset(wd[...].astype(F32))
            om = 1.0 - jnp.concatenate([g_v[rows, :]] * (D // 128), axis=1)
            db = om * dout_v[rows, :].astype(F32)
            db11, db22 = db[:hr, :hd].astype(BF16), db[hr:, hd:].astype(BF16)
            dbs = _tset(db)
            dh11, dh12, dh21, dh22 = _strassen(_lhs7(wd11, wd22, wds_), _rhs7_t(db11, db22, dbs), _NT, swap=True)
            w11, w22 = w[:hd, :FC], w[hd:, FC:]
            ws = _nset(w[...].astype(F32))
            x11, x22 = x_v[top, :hd], x_v[bot, hd:]
            xs = _nset(x_v[rows, :].astype(F32))
            g1, u1, g2, u2 = _strassen(_lhs7(x11, x22, xs), _rhs7(w11, w22, ws), _NN)
            h = jnp.concatenate([g1 * u1, g2 * u2], axis=0)
            hs = _nset(h)
            h11, h22 = h[:hr, :hf].astype(BF16), h[hr:, hf:].astype(BF16)
            bnew = _full(*_strassen(_lhs7(h11, h22, hs), _rhs7(wd11, wd22, wds_), _NN))
            bacc[rows, :] = jnp.where(c > 0, bacc[rows, :], 0.0) + bnew
            dnew = _full(*_strassen(_lhs7(db11, db22, dbs), _rhs7(h11, h22, hs), _TN, swap=True))
            dtot = jnp.where(r > 0, dwd_acc[...], 0.0) + dnew
            dwd_acc[...] = dtot
            stg_d[slot] = dtot.astype(BF16)

            dht = jnp.concatenate([dh11, dh12], axis=1)
            dhb = jnp.concatenate([dh21, dh22], axis=1)
            dgu = _full(dht * u1, dht * g1, dhb * u2, dhb * g2)
            gs = _tset(dgu)
            d11, d22 = dgu[:hr, :FC].astype(BF16), dgu[hr:, FC:].astype(BF16)
            xnew = _full(*_strassen(_lhs7(w11, w22, ws), _rhs7_t(d11, d22, gs), _NT, swap=True))
            dxacc[rows, :] = jnp.where(c > 0, dxacc[rows, :], 0.0) + xnew
            wnew = _full(*_strassen(_lhs7(d11, d22, gs), _rhs7(x11, x22, xs), _TN, swap=True))
            wtot = jnp.where(r > 0, dwgu_acc[...], 0.0) + wnew
            dwgu_acc[...] = wtot
            stg_gu[slot] = wtot.astype(BF16)

            @pl.when(r == NR4 - 1)
            def _():
                for cp in dw_cps(c, slot):
                    cp.start()

            return carry

        _loop("P4", NF * NR4, p4_body)

        def fin_cps(r, slot):
            return (pltpu.make_async_copy(stg_out.at[slot], out_hbm.at[_rows(r)], sem_fin.at[slot, 0]),
                    pltpu.make_async_copy(stg_dx.at[slot], dx_hbm.at[_rows(r)], sem_fin.at[slot, 1]))

        def p5_body(r, dgw):
            slot = r % 2

            @pl.when(r >= 2)
            def _():
                for cp in fin_cps(r - 2, slot):
                    cp.wait()

            rows = _rows(r)
            hd, hr, hq = D // 2, R // 2, 3 * D // 2
            sa = _Strassen(_lhs7(ot_v[r, :hd, :hr], ot_v[r, hd:, hr:], _tset(ot_v[r].astype(F32))),
                           _rhs7(wo_v[:hd, :hd], wo_v[hd:, hd:], [wos_v[i] for i in range(5)]), _TN)
            dqkv_t = jnp.concatenate([dqkvt_v[r, 0:D, :], dqkvt_v[r, D:2 * D, :] * LN2,
                                      dqkvt_v[r, 2 * D:3 * D, :]], axis=0)
            sx = _Strassen(_lhs7(wqkv_v[:hd, :hq], wqkv_v[hd:, hq:], [wqs_v[i] for i in range(5)]),
                           _rhs7(dqkv_t[:hq, :hr].astype(BF16), dqkv_t[hq:, hr:].astype(BF16), _nset(dqkv_t)),
                           _TT, swap=True)
            sx.prod(2)
            a = _full(*sa.blocks())
            b = bacc[rows, :]
            g1 = g_v[rows, :]
            gate = jnp.concatenate([g1] * (D // 128), axis=1)
            stg_out[slot] = (gate * a + (1.0 - gate) * b).astype(BF16)
            fin_cps(r, slot)[0].start()
            dg = jnp.sum(dout_v[rows, :].astype(F32) * (a - b), axis=-1, keepdims=True)
            g0 = g1[:, 0:1]
            dz = dg * g0 * (1.0 - g0)
            dxa = _full(*sx.blocks())
            dx = dxa + dxacc[rows, :] + dz * gw
            stg_dx[slot] = dx.astype(BF16)
            fin_cps(r, slot)[1].start()
            return dgw + jnp.sum(dz * x_v[rows, :].astype(F32), axis=0, keepdims=True)

        dgw = _loop("P5", NR, p5_body, jnp.zeros((1, D), F32))
        dgw_ref[...] = dgw.astype(BF16)

        dwo_cp.wait()
        for j in range(n_j - 2, n_j):
            q_cp(j, j % 2).wait()
        for c in range(NF - 2, NF):
            for cp in dw_cps(c, c % 2):
                cp.wait()
        for r in range(NR - 2, NR):
            for cp in fin_cps(r, r % 2):
                cp.wait()

    pl.run_scoped(
        tail_scope,
        pltpu.VMEM((S, D), F32), pltpu.VMEM((S, D), F32),
        pltpu.VMEM((2, D, 2 * FC), BF16), pltpu.VMEM((2, FC, D), BF16),
        pltpu.VMEM((D, 2 * FC), F32), pltpu.VMEM((FC, D), F32),
        pltpu.VMEM((2, D, 2 * FC), BF16), pltpu.VMEM((2, FC, D), BF16),
        pltpu.VMEM((2, D, R), BF16), pltpu.VMEM((D, D), BF16),
        pltpu.VMEM((2, R, D), BF16), pltpu.VMEM((2, R, D), BF16),
        pltpu.SemaphoreType.DMA((2, 3)), pltpu.SemaphoreType.DMA((2, 3)),
        pltpu.SemaphoreType.DMA((3,)), pltpu.SemaphoreType.DMA((2, 2)),
    )


@jax.jit
def pallas_gated_mix__softmax_full_mha__glu_gated_bilinear__prompt_kernel(
    A_x: jax.Array,
    A_wqkv: jax.Array,
    A_wo: jax.Array,
    B_x: jax.Array,
    B_w_gate: jax.Array,
    B_w_up: jax.Array,
    B_w_down: jax.Array,
    gate_w: jax.Array,
    grad_out: jax.Array,
):
    del B_x
    hbm = pl.BlockSpec(memory_space=pl.ANY)
    vmem = pl.BlockSpec(memory_space=pltpu.VMEM)
    sds = jax.ShapeDtypeStruct
    outs = pl.pallas_call(
        _kernel,
        in_specs=[hbm, hbm, hbm, hbm, hbm, hbm, vmem, hbm],
        out_specs=(hbm, hbm, hbm, hbm, hbm, hbm, hbm, vmem),
        out_shape=(sds((S, D), BF16), sds((S, D), BF16), sds((D, 3 * D), BF16), sds((D, D), BF16),
                   sds((D, F), BF16), sds((D, F), BF16), sds((F, D), BF16), sds((1, D), BF16)),
        scratch_shapes=[
            pltpu.VMEM((S, D), BF16),
            pltpu.VMEM((S, D), BF16),
            pltpu.VMEM((D, 3 * D), BF16),
            pltpu.VMEM((D, D), BF16),
            pltpu.VMEM((5, D // 2, 3 * D // 2), BF16),
            pltpu.VMEM((5, D // 2, D // 2), BF16),
            pltpu.VMEM((S, 128), F32),
            pltpu.VMEM((NR, 8, R), F32),
            pltpu.VMEM((NR, D, R), BF16),
            pltpu.VMEM((NR, 3 * D, R), F32),
            pltpu.SemaphoreType.DMA((2 * NR + 2,)),
        ],
        compiler_params=pltpu.CompilerParams(vmem_limit_bytes=127 * 1024 * 1024),
    )(A_x.reshape(S, D), A_wqkv, A_wo, B_w_gate, B_w_up, B_w_down,
      jnp.broadcast_to(gate_w.astype(F32), (8, D)), grad_out.reshape(S, D))
    out, dx, dwqkv, dwo, dwg, dwu, dwd, dgw = outs
    return (out.reshape(1, S, D), dx.reshape(1, S, D), dwqkv, dwo, dwg, dwu, dwd, dgw.reshape(D))
```
